```python
import jax
import jax.numpy as jnp

def _softmax(x, axis=-1):
    return jax.nn.softmax(x, axis=axis)
def _gelu(x):
    return jax.nn.gelu(x, approximate=True)
def _silu(x):
    return jax.nn.silu(x)
def _sigmoid(x):
    return jax.nn.sigmoid(x)
def _layernorm(x, axis=-1, eps=1e-5):
    m = jnp.mean(x, axis=axis, keepdims=True)
    v = jnp.var(x, axis=axis, keepdims=True)
    return (x - m) / jnp.sqrt(v + eps)
def _scatter_add(tgt, idx, src, axis=0):
    return tgt.at[idx].add(src)
def _segment_sum(src, seg, n):
    return jax.ops.segment_sum(src, seg, n)
class _Rng:
    def __init__(self, key):
        self._k = key
    def _next(self):
        self._k, sub = jax.random.split(self._k)
        return sub
    def normal(self, shape):
        return jax.random.normal(self._next(), shape, dtype=jnp.bfloat16)
    def randint(self, lo, hi, shape):
        return jax.random.randint(self._next(), shape, lo, hi, dtype=jnp.int32)
    def uniform(self, shape, lo=0.0, hi=1.0):
        return jax.random.uniform(self._next(), shape, jnp.bfloat16, lo, hi)
    def permutation(self, n):
        return jax.random.permutation(self._next(), n)


kernel_name = 'sequential_preLN__spectral_gfnet__swiglu_ffn__prompt'

def _fwd_setup_inputs():
    _rng = _Rng(jax.random.key(int.from_bytes(__import__("os").urandom(4), "little")))
    _w = (lambda a: (lambda t: t.astype(jnp.bfloat16) if jnp.issubdtype(t.dtype, jnp.floating) else t)(jnp.asarray(a)))
    def _A_setup():
        B, S, D = 1, 2048, 576
        Df = D // 2 + 1
        return {
            "x": _w((lambda *s: _rng.normal(s) * 0.05)(B, S, D)),
            "w_r": _w((lambda *s: _rng.normal(s) * 0.05)(S, Df) * 0.02),
            "w_i": _w((lambda *s: _rng.normal(s) * 0.05)(S, Df) * 0.02),
        }
    _A_in = _A_setup()

    def _B_setup():
        B, S, D, F = 1, 2048, 576, 4608
        return {
            "x": _w((lambda *s: _rng.normal(s) * 0.05)(B, S, D)),
            "w_gate": _w((lambda *s: _rng.normal(s) * 0.05)(D, F)),
            "w_up": _w((lambda *s: _rng.normal(s) * 0.05)(D, F)),
            "w_down": _w((lambda *s: _rng.normal(s) * 0.05)(F, D)),
        }
    _B_in = _B_setup()

    return {
        "A_x": _A_in["x"],
        "A_w_r": _A_in["w_r"],
        "A_w_i": _A_in["w_i"],
        "B_x": _B_in["x"],
        "B_w_gate": _B_in["w_gate"],
        "B_w_up": _B_in["w_up"],
        "B_w_down": _B_in["w_down"],
    }

def _fwd_reference(A_x, A_w_r, A_w_i, B_x, B_w_gate, B_w_up, B_w_down):
    def _A_ref(x, w_r, w_i):
        B, S, D = x.shape
        X = (lambda x, axes=(-2,-1): jnp.fft.rfft2(x.astype(jnp.float32), axes=axes))(x, axes=(-2, -1))
        W = w_r + 1j * w_i
        X = X * W
        y = (lambda x, s, axes=(-2,-1): jnp.fft.irfft2(x, s=s, axes=axes).astype(jnp.bfloat16))(X, (S, D), axes=(-2, -1))
        return y

    def _B_ref(x, w_gate, w_up, w_down):
        g = _silu(x @ w_gate)
        u = x @ w_up
        return (g * u) @ w_down

    x = A_x
    h = x + _A_ref(_layernorm(x, axis=-1), A_w_r, A_w_i)
    h2 = h + _B_ref(_layernorm(h, axis=-1), B_w_gate, B_w_up, B_w_down)
    return h2


def setup_inputs():
    _inp = _fwd_setup_inputs()
    _gk = jax.random.fold_in(jax.random.key(int.from_bytes(__import__("os").urandom(4), "little")), 2**31 - 1)
    _shapes = [[1, 2048, 576]]
    _dtypes = ['bfloat16']
    _gks = jax.random.split(_gk, len(_shapes))
    _gs = [jax.random.normal(k, s, dtype=jnp.dtype(d)) * 0.05 for k, s, d in zip(_gks, _shapes, _dtypes)]
    _inp["grad_out"] = _gs[0]
    return _inp

def reference(A_x, A_w_r, A_w_i, B_w_gate, B_w_up, B_w_down, B_x, grad_out):
    _const = dict(B_x=B_x)
    def _f(*_d):
        return _fwd_reference(**{'A_x': _d[0], 'A_w_r': _d[1], 'A_w_i': _d[2], 'B_w_gate': _d[3], 'B_w_up': _d[4], 'B_w_down': _d[5], **_const})
    _out, _vjp = jax.vjp(_f, A_x, A_w_r, A_w_i, B_w_gate, B_w_up, B_w_down)
    _grads = _vjp(grad_out)
    _out0 = jnp.asarray(_out)
    return (_out0, *[jnp.asarray(_g) for _g in _grads])
```

```python
import functools
import math

import jax
import jax.numpy as jnp
import numpy as np
import jax.experimental.pallas as pl
import jax.experimental.pallas.tpu as pltpu

F32 = jnp.float32
BF16 = jnp.bfloat16
U32 = jnp.uint32

S = 2048
D = 576
FF = 4608
DF = D // 2 + 1
H = D // 2
NE = 145
RE = 160
RO = 144
FR = RE + RO
N1 = 16
N2 = 128
EPS = 1e-5

TM = 512
TF = 512
FC = 512
RC = 16


@functools.lru_cache(maxsize=None)
def _tables():
    d2 = np.arange(H)[None, :]
    cf = np.full((DF,), 2.0)
    cf[0] = 1.0
    cf[DF - 1] = 1.0
    scale = cf / (S * D)

    def trig(fs):
        ang = 2.0 * np.pi * ((fs[:, None] * d2) % D) / D
        cs, sn = np.cos(ang), np.sin(ang)
        sn[(fs == 0) | (fs == DF - 1), :] = 0.0
        return cs, sn

    fe = np.arange(0, DF, 2)
    fo = np.arange(1, DF, 2)
    ce, se = trig(fe)
    co, so = trig(fo)
    fd = np.zeros((2 * FR, H), np.float64)
    fd[0:NE] = ce
    fd[RE:RE + NE] = -se
    fd[2 * RE:2 * RE + RO] = co
    fd[2 * RE + RO:] = -so
    gd = np.zeros((H, 2 * FR), np.float64)
    gd[:, 0:NE] = (ce * scale[fe][:, None]).T
    gd[:, RE:RE + NE] = (-se * scale[fe][:, None]).T
    gd[:, 2 * RE:2 * RE + RO] = (co * scale[fo][:, None]).T
    gd[:, 2 * RE + RO:] = (-so * scale[fo][:, None]).T
    mf = np.zeros((N1, 2 * N2, 2 * N2), np.float64)
    k2 = np.arange(N2)[:, None]
    n2 = np.arange(N2)[None, :]
    for k1 in range(N1):
        a = 2.0 * np.pi * ((n2 * (k1 + N1 * k2)) % S) / S
        mr, mi = np.cos(a), -np.sin(a)
        mf[k1, :N2, :N2] = mr
        mf[k1, :N2, N2:] = -mi
        mf[k1, N2:, :N2] = mi
        mf[k1, N2:, N2:] = mr
    mt = np.transpose(mf, (0, 2, 1))
    cd = np.zeros((FR, N2), np.float64)
    cd[0:NE, :] = scale[fe][:, None]
    cd[RE:, :] = scale[fo][:, None]
    to = lambda a: np.asarray(a, np.float32).astype(jnp.bfloat16)
    return to(fd), to(gd), to(mt), np.asarray(cd, np.float32)


def _cmul_const(v, c, s):
    vr, vi = v
    eps = 1e-12
    if abs(s) < eps:
        if abs(c - 1.0) < eps:
            return vr, vi
        if abs(c + 1.0) < eps:
            return -vr, -vi
    if abs(c) < eps:
        if abs(s - 1.0) < eps:
            return -vi, vr
        if abs(s + 1.0) < eps:
            return vi, -vr
    if abs(abs(c) - abs(s)) < eps:
        a = (vr - vi) if (c * s > 0) else (vr + vi)
        b = (vi + vr) if (c * s > 0) else (vi - vr)
        return a * c, b * c
    return vr * c - vi * s, vi * c + vr * s


def _fft_list(vals, sign):
    n = len(vals)
    if n == 1:
        return vals
    ev = _fft_list(vals[0::2], sign)
    od = _fft_list(vals[1::2], sign)
    out = [None] * n
    for k in range(n // 2):
        ang = sign * 2.0 * math.pi * k / n
        tr, ti = _cmul_const(od[k], math.cos(ang), math.sin(ang))
        er, ei = ev[k]
        out[k] = (er + tr, ei + ti)
        out[k + n // 2] = (er - tr, ei - ti)
    return out


def _dot(a, b):
    return jnp.dot(a, b, preferred_element_type=F32)


def _dot_nt(a, b):
    return jax.lax.dot_general(a, b, (((1,), (1,)), ((), ())),
                               preferred_element_type=F32)


def _kernel(x_hbm, wr_hbm, wi_hbm, wg_hbm, wu_hbm, wd_hbm, go_hbm,
            fd_hbm, gd_hbm, mt_hbm, cd_hbm,
            out_hbm, dx_hbm, dwr_hbm, dwi_hbm, dwg_hbm, dwu_hbm, dwd_hbm,
            x_v, go_v, wg_v, wu_v, wd_v,
            fd_v, gd_v, mt_v, cd_v, wr_v, wi_v,
            zbuf, tbuf, xbuf, vbuf, wp, wf, wtmp,
            h_v, hnt_v, hnr_v, gor_v, dh_v, out_v, dx_v, oacc, hacc,
            acc, stage, st_v,
            sem_in, sem_out, sem_w, sem_dw, sem_x, sem_wi):
    nt = S // TM
    nc = FF // FC

    def x_copy(i):
        r0 = pl.multiple_of(i * TM, TM)
        return pltpu.make_async_copy(x_hbm.at[:, pl.ds(r0, TM)],
                                     x_v.at[:, pl.ds(r0, TM)], sem_x.at[i])

    def w_copies(c):
        c0 = pl.multiple_of(c * FC, FC)
        return [pltpu.make_async_copy(h.at[:, pl.ds(c0, FC)],
                                      v.at[:, pl.ds(c0, FC)], sem_wi.at[j, c])
                for j, (h, v) in enumerate(((wg_hbm, wg_v), (wu_hbm, wu_v),
                                            (wd_hbm, wd_v)))]

    in_pairs = [(fd_hbm, fd_v), (wr_hbm, wr_v), (wi_hbm, wi_v),
                (mt_hbm, mt_v), (cd_hbm, cd_v), (gd_hbm, gd_v),
                (go_hbm, go_v)]
    cps = [pltpu.make_async_copy(s, d, sem_in.at[i])
           for i, (s, d) in enumerate(in_pairs)]
    (cp_fd, cp_wr, cp_wi, cp_mt, cp_cd, cp_gd, cp_go) = cps
    x_copy(0).start()
    cp_fd.start()
    x_copy(1).start()
    wf[...] = jnp.zeros(wf.shape, U32)

    def ln_stats(v):
        mu = jnp.mean(v, axis=0, keepdims=True)
        c = v - mu
        var = jnp.mean(c * c, axis=0, keepdims=True)
        rs = jax.lax.rsqrt(var + EPS)
        return c * rs, mu, rs

    def rfft_d(i, v):
        lo, hi = v[0:H], v[H:D]
        ze = _dot(fd_v[0:2 * RE, :], (lo + hi).astype(BF16))
        zo = _dot(fd_v[2 * RE:, :], (lo - hi).astype(BF16))
        for b in range(TM // N2):
            n1 = i * (TM // N2) + b
            cols = slice(b * N2, (b + 1) * N2)
            zbuf[n1, 0:RE, 0:N2] = ze[0:RE, cols]
            zbuf[n1, 0:RE, N2:2 * N2] = ze[RE:2 * RE, cols]
            zbuf[n1, RE:FR, 0:N2] = zo[0:RO, cols]
            zbuf[n1, RE:FR, N2:2 * N2] = zo[RO:2 * RO, cols]

    def irfft_d(r0):
        e = _dot(gd_v[:, 0:2 * RE], vbuf[0:2 * RE, pl.ds(r0, TM)])
        o = _dot(gd_v[:, 2 * RE:], vbuf[2 * RE:, pl.ds(r0, TM)])
        return jnp.concatenate([e + o, e - o], axis=0)

    def dft16_fwd():
        def body(j, _):
            r = pl.multiple_of(j * RC, RC)
            vals = [(zbuf[n1, pl.ds(r, RC), 0:N2],
                     zbuf[n1, pl.ds(r, RC), N2:2 * N2]) for n1 in range(N1)]
            res = _fft_list(vals, -1.0)
            for k1 in range(N1):
                tbuf[k1, pl.ds(r, RC), 0:N2] = res[k1][0].astype(BF16)
                tbuf[k1, pl.ds(r, RC), N2:2 * N2] = res[k1][1].astype(BF16)
            return 0
        jax.lax.fori_loop(0, FR // RC, body, 0)

    def dft16_inv():
        def body(j, _):
            r = pl.multiple_of(j * RC, RC)
            vals = [(zbuf[k1, pl.ds(r, RC), 0:N2],
                     zbuf[k1, pl.ds(r, RC), N2:2 * N2]) for k1 in range(N1)]
            res = _fft_list(vals, 1.0)
            odd = j >= RE // RC
            r_re = pl.multiple_of(jnp.where(odd, r + RE, r), RC)
            r_im = pl.multiple_of(jnp.where(odd, r + FR, r + RE), RC)
            for n1 in range(N1):
                vbuf[pl.ds(r_re, RC), n1 * N2:(n1 + 1) * N2] = (
                    res[n1][0].astype(BF16))
                vbuf[pl.ds(r_im, RC), n1 * N2:(n1 + 1) * N2] = (
                    res[n1][1].astype(BF16))
            return 0
        jax.lax.fori_loop(0, FR // RC, body, 0)

    hi_mask = jnp.uint32(0xFFFF0000)

    def pack2(re_f32, im_f32):
        re_b = pltpu.bitcast(re_f32, U32)
        im_b = pltpu.bitcast(im_f32, U32)
        return (re_b & hi_mask) | (im_b >> 16)

    def unpack2(w):
        return (pltpu.bitcast(w & hi_mask, F32),
                pltpu.bitcast(w << 16, F32))

    def perm_a(i):
        r0 = pl.multiple_of(i * TM, TM)
        wf[0:DF, pl.ds(r0, TM)] = pack2(
            wr_v[:, pl.ds(r0, TM)].astype(F32),
            wi_v[:, pl.ds(r0, TM)].astype(F32))
        for j in range(3):
            wtmp[j, pl.ds(r0, TM), :] = (
                wf[j * 128:(j + 1) * 128, pl.ds(r0, TM)].T)

    def perm_b(k1):
        blks = [wtmp[j, pl.ds(k1, N2, stride=N1), :].T for j in range(3)]
        blks[2] = blks[2][0:2 * RE - 256]
        return jnp.concatenate(blks, axis=0)

    def load_w(k1):
        return jnp.concatenate([wp[k1, pl.ds(0, RE, stride=2), :],
                                wp[k1, pl.ds(1, RO, stride=2), :]], axis=0)

    def unperm_b(k1, w):
        wp[k1, pl.ds(0, RE, stride=2), :] = w[0:RE]
        wp[k1, pl.ds(1, RO, stride=2), :] = w[RE:FR]
        w = jnp.concatenate([wp[k1], jnp.zeros((384 - 2 * RE, N2), U32)],
                            axis=0)
        for j in range(3):
            wtmp[j, pl.ds(k1, N2, stride=N1), :] = w[j * 128:(j + 1) * 128].T

    def unperm_a(i):
        r0 = pl.multiple_of(i * TM, TM)
        for j in range(3):
            wf[j * 128:(j + 1) * 128, pl.ds(r0, TM)] = (
                wtmp[j, pl.ds(r0, TM), :].T)
        re, im = unpack2(wf[0:DF, pl.ds(r0, TM)])
        wr_v[:, pl.ds(r0, TM)] = re.astype(BF16)
        wi_v[:, pl.ds(r0, TM)] = im.astype(BF16)

    def dws_copies(i):
        r0 = pl.multiple_of(i * TM, TM)
        return [pltpu.make_async_copy(v.at[:, pl.ds(r0, TM)],
                                      o.at[:, pl.ds(r0, TM)], sem_w.at[j])
                for j, (v, o) in enumerate(((wr_v, dwr_hbm),
                                            (wi_v, dwi_hbm)))]

    cp_fd.wait()

    for i in range(nt):
        x_copy(i).wait()
        if i == 0:
            for t in range(2, nt):
                x_copy(t).start()
            cp_wr.start()
            cp_wi.start()
        if i == 2:
            cp_mt.start()
        if i == 3:
            cp_go.start()
            cp_gd.start()
            cp_cd.start()
        xt = x_v[:, i * TM:(i + 1) * TM].astype(F32)
        xn, mu, rs = ln_stats(xt)
        st_v[0:1, i * TM:(i + 1) * TM] = mu
        st_v[1:2, i * TM:(i + 1) * TM] = rs
        rfft_d(i, xn.astype(BF16).astype(F32))
        if i == nt - 2:
            cp_wr.wait()
            cp_wi.wait()
        if i >= nt - 2:
            for t in range((i - (nt - 2)) * nt // 2, (i - (nt - 3)) * nt // 2):
                perm_a(t)

    dft16_fwd()

    cp_mt.wait()

    def p1c(k1, with_go):
        xk = _dot(tbuf[k1], mt_v[k1])
        xbuf[k1] = xk
        xr, xi = xk[:, 0:N2], xk[:, N2:2 * N2]
        wp[k1] = perm_b(k1)
        wr, wi = unpack2(load_w(k1))
        y = jnp.concatenate([xr * wr - xi * wi, xr * wi + xi * wr], axis=1)
        zbuf[k1] = _dot_nt(y.astype(BF16), mt_v[k1])
        if with_go:
            t0 = pl.multiple_of((k1 - N1 // 2) * 2 * N2, 2 * N2)
            gor_v[pl.ds(t0, 2 * N2), :] = (
                go_v[:, pl.ds(t0, 2 * N2)].astype(F32).T.astype(BF16))
        return 0
    jax.lax.fori_loop(0, N1 // 2, lambda k, _: p1c(k, False), 0, unroll=4)
    cp_go.wait()
    for c in range(nc):
        for cp in w_copies(c):
            cp.start()
    jax.lax.fori_loop(N1 // 2, N1, lambda k, _: p1c(k, True), 0, unroll=4)

    dft16_inv()

    cp_gd.wait()
    cp_cd.wait()

    def p2a(i, _):
        r0 = pl.multiple_of(i * TM, TM)
        xt = x_v[:, pl.ds(r0, TM)].astype(F32)
        y = irfft_d(r0)
        h = (xt + y.astype(BF16).astype(F32)).astype(BF16)
        h_v[:, pl.ds(r0, TM)] = h
        h = h.astype(F32)
        hn, mu, rs = ln_stats(h)
        st_v[2:3, pl.ds(r0, TM)] = mu
        st_v[3:4, pl.ds(r0, TM)] = rs
        hnt_v[:, pl.ds(r0, TM)] = hn.astype(BF16)
        hnr_v[pl.ds(r0, TM), :] = hn.T.astype(BF16)
        return 0
    jax.lax.fori_loop(0, nt, p2a, 0, unroll=True)

    def dw_copies(c):
        c0 = pl.multiple_of(c * FC, FC)
        return [pltpu.make_async_copy(stage.at[c % 2, j],
                                      o.at[:, pl.ds(c0, FC)],
                                      sem_dw.at[j, c])
                for j, o in enumerate((dwg_hbm, dwu_hbm, dwd_hbm))]

    def chunk(c, _):
        c0 = pl.multiple_of(c * FC, FC)
        slot = c % 2
        for cp in w_copies(c):
            cp.wait()

        @pl.when(c >= 2)
        def _():
            for cp in dw_copies(c - 2):
                cp.wait()

        def tile(i, _):
            r0 = pl.multiple_of(i * TF, TF)
            wg = wg_v[:, pl.ds(c0, FC)]
            wu = wu_v[:, pl.ds(c0, FC)]
            wd = wd_v[:, pl.ds(c0, FC)]
            hn_r = hnr_v[pl.ds(r0, TF), :]
            a = _dot(hn_r, wg)
            u = _dot(hn_r, wu)
            dgu = _dot(gor_v[pl.ds(r0, TF), :], wd)
            s = jax.nn.sigmoid(a)
            g = a * s
            gu = (g * u).astype(BF16)
            du = (dgu * g).astype(BF16)
            da = (dgu * u * (s * (1.0 + a * (1.0 - s)))).astype(BF16)
            oacc[:, pl.ds(r0, TF)] = _dot_nt(wd, gu) + jnp.where(
                c > 0, oacc[:, pl.ds(r0, TF)], 0.0)
            hacc[:, pl.ds(r0, TF)] = (
                _dot_nt(wg, da) + _dot_nt(wu, du)
                + jnp.where(c > 0, hacc[:, pl.ds(r0, TF)], 0.0))
            hn_t = hnt_v[:, pl.ds(r0, TF)]
            parts = (_dot(hn_t, da), _dot(hn_t, du),
                     _dot(go_v[:, pl.ds(r0, TF)], gu))
            for j, p in enumerate(parts):
                p = p + jnp.where(i > 0, acc[j], 0.0)
                acc[j] = p
                stage[slot, j] = p.astype(BF16)
            return 0
        jax.lax.fori_loop(0, S // TF, tile, 0)
        for cp in dw_copies(c):
            cp.start()
        return 0
    jax.lax.fori_loop(0, nc, chunk, 0)

    def p2c(i, _):
        r0 = pl.multiple_of(i * TM, TM)
        h = h_v[:, pl.ds(r0, TM)].astype(F32)
        out_v[:, pl.ds(r0, TM)] = (h + oacc[:, pl.ds(r0, TM)]).astype(BF16)
        pltpu.make_async_copy(out_v.at[:, pl.ds(r0, TM)],
                              out_hbm.at[:, pl.ds(r0, TM)],
                              sem_out.at[0]).start()
        rs = st_v[3:4, pl.ds(r0, TM)]
        hn = (h - st_v[2:3, pl.ds(r0, TM)]) * rs
        dhn = hacc[:, pl.ds(r0, TM)]
        m1 = jnp.mean(dhn, axis=0, keepdims=True)
        m2 = jnp.mean(dhn * hn, axis=0, keepdims=True)
        dh = go_v[:, pl.ds(r0, TM)].astype(F32) + rs * (dhn - m1 - hn * m2)
        dh_v[:, pl.ds(r0, TM)] = dh
        rfft_d(i, dh)
        return 0
    jax.lax.fori_loop(0, nt, p2c, 0, unroll=True)

    dft16_fwd()

    def p3c(k1, _):
        gk = _dot(tbuf[k1], mt_v[k1])
        gr, gi = gk[:, 0:N2], gk[:, N2:2 * N2]
        xk = xbuf[k1]
        xr, xi = xk[:, 0:N2], xk[:, N2:2 * N2]
        wr, wi = unpack2(load_w(k1))
        cd = cd_v[...]
        dwr = ((gr * xr + gi * xi) * cd).astype(BF16).astype(F32)
        dwi = ((gi * xr - gr * xi) * cd).astype(BF16).astype(F32)
        unperm_b(k1, pack2(dwr, dwi))
        y = jnp.concatenate([gr * wr + gi * wi, gi * wr - gr * wi], axis=1)
        zbuf[k1] = _dot_nt(y.astype(BF16), mt_v[k1])
        return 0
    jax.lax.fori_loop(0, N1, p3c, 0, unroll=4)


    pltpu.make_async_copy(out_v, out_hbm, sem_out.at[0]).wait()
    for c in range(nc - 2, nc):
        for cp in dw_copies(c):
            cp.wait()

    dft16_inv()

    for i in range(nt):
        r0 = i * TM
        xt = x_v[:, pl.ds(r0, TM)].astype(F32)
        rs = st_v[1:2, pl.ds(r0, TM)]
        xn = (xt - st_v[0:1, pl.ds(r0, TM)]) * rs
        dxn = irfft_d(r0)
        m1 = jnp.mean(dxn, axis=0, keepdims=True)
        m2 = jnp.mean(dxn * xn, axis=0, keepdims=True)
        dx = dh_v[:, pl.ds(r0, TM)] + rs * (dxn - m1 - xn * m2)
        dx_v[:, pl.ds(r0, TM)] = dx.astype(BF16)
        pltpu.make_async_copy(dx_v.at[:, pl.ds(r0, TM)],
                              dx_hbm.at[:, pl.ds(r0, TM)],
                              sem_out.at[1]).start()
        if i < 2:
            for t in range(i * nt // 2, (i + 1) * nt // 2):
                unperm_a(t)
                for cp in dws_copies(t):
                    cp.start()

    pltpu.make_async_copy(wr_v, dwr_hbm, sem_w.at[0]).wait()
    pltpu.make_async_copy(wi_v, dwi_hbm, sem_w.at[1]).wait()
    pltpu.make_async_copy(dx_v, dx_hbm, sem_out.at[1]).wait()


@jax.jit
def pallas_sequential_preLN__spectral_gfnet__swiglu_ffn__prompt_kernel(
    A_x: jax.Array,
    A_w_r: jax.Array,
    A_w_i: jax.Array,
    B_x: jax.Array,
    B_w_gate: jax.Array,
    B_w_up: jax.Array,
    B_w_down: jax.Array,
    grad_out: jax.Array,
):
    del B_x
    fd, gd, mt, cd = _tables()
    nt = S // TM

    any_spec = pl.BlockSpec(memory_space=pl.ANY)

    outs = pl.pallas_call(
        _kernel,
        in_specs=[any_spec] * 11,
        out_specs=[any_spec] * 7,
        out_shape=[
            jax.ShapeDtypeStruct((D, S), BF16),
            jax.ShapeDtypeStruct((D, S), BF16),
            jax.ShapeDtypeStruct((DF, S), BF16),
            jax.ShapeDtypeStruct((DF, S), BF16),
            jax.ShapeDtypeStruct((D, FF), BF16),
            jax.ShapeDtypeStruct((D, FF), BF16),
            jax.ShapeDtypeStruct((D, FF), BF16),
        ],
        scratch_shapes=[
            pltpu.VMEM((D, S), BF16),
            pltpu.VMEM((D, S), BF16),
            pltpu.VMEM((D, FF), BF16),
            pltpu.VMEM((D, FF), BF16),
            pltpu.VMEM((D, FF), BF16),
            pltpu.VMEM((2 * FR, H), BF16),
            pltpu.VMEM((H, 2 * FR), BF16),
            pltpu.VMEM((N1, 2 * N2, 2 * N2), BF16),
            pltpu.VMEM((FR, N2), F32),
            pltpu.VMEM((DF, S), BF16),
            pltpu.VMEM((DF, S), BF16),
            pltpu.VMEM((N1, FR, 2 * N2), F32),
            pltpu.VMEM((N1, FR, 2 * N2), BF16),
            pltpu.VMEM((N1, FR, 2 * N2), F32),
            pltpu.VMEM((2 * FR, S), BF16),
            pltpu.VMEM((N1, 2 * RE, N2), U32),
            pltpu.VMEM((384, S), U32),
            pltpu.VMEM((3, S, 128), U32),
            pltpu.VMEM((D, S), BF16),
            pltpu.VMEM((D, S), BF16),
            pltpu.VMEM((S, D), BF16),
            pltpu.VMEM((S, D), BF16),
            pltpu.VMEM((D, S), F32),
            pltpu.VMEM((D, S), BF16),
            pltpu.VMEM((D, S), BF16),
            pltpu.VMEM((D, S), F32),
            pltpu.VMEM((D, S), F32),
            pltpu.VMEM((3, D, FC), F32),
            pltpu.VMEM((2, 3, D, FC), BF16),
            pltpu.VMEM((8, S), F32),
            pltpu.SemaphoreType.DMA((7,)),
            pltpu.SemaphoreType.DMA((2,)),
            pltpu.SemaphoreType.DMA((2,)),
            pltpu.SemaphoreType.DMA((3, FF // FC)),
            pltpu.SemaphoreType.DMA((nt,)),
            pltpu.SemaphoreType.DMA((3, FF // FC)),
        ],
        compiler_params=pltpu.CompilerParams(
            vmem_limit_bytes=120 * 1024 * 1024),
    )(A_x.reshape(S, D).T, A_w_r.T, A_w_i.T, B_w_gate, B_w_up, B_w_down.T,
      grad_out.reshape(S, D).T, fd, gd, mt, cd)
    out_t, dx_t, dwr_t, dwi_t, dwg, dwu, dwd_t = outs
    return (out_t.T.reshape(1, S, D), dx_t.T.reshape(1, S, D), dwr_t.T,
            dwi_t.T, dwg, dwu, dwd_t.T)
```
